```python
import os as _os
_os.environ.setdefault("JAX_PLATFORMS", "cpu")
import jax
import jax.numpy as jnp

def _softmax(x, axis=-1):
    return jax.nn.softmax(x, axis=axis)
def _gelu(x):
    return jax.nn.gelu(x, approximate=True)
def _silu(x):
    return jax.nn.silu(x)
def _sigmoid(x):
    return jax.nn.sigmoid(x)
def _layernorm(x, axis=-1, eps=1e-5):
    m = jnp.mean(x, axis=axis, keepdims=True)
    v = jnp.var(x, axis=axis, keepdims=True)
    return (x - m) / jnp.sqrt(v + eps)
def _scatter_add(tgt, idx, src, axis=0):
    return tgt.at[idx].add(src)
def _segment_sum(src, seg, n):
    return jax.ops.segment_sum(src, seg, n)
class _Rng:
    def __init__(self, key):
        self._k = key
    def _next(self):
        self._k, sub = jax.random.split(self._k)
        return sub
    def normal(self, shape):
        return jax.random.normal(self._next(), shape, dtype=jnp.bfloat16)
    def randint(self, lo, hi, shape):
        return jax.random.randint(self._next(), shape, lo, hi, dtype=jnp.int32)
    def uniform(self, shape, lo=0.0, hi=1.0):
        return jax.random.uniform(self._next(), shape, jnp.bfloat16, lo, hi)
    def permutation(self, n):
        return jax.random.permutation(self._next(), n)


kernel_name = 'standalone__mha_block_cached__near_ridge'

def setup_inputs():
    _rng = _Rng(jax.random.key(int.from_bytes(__import__("os").urandom(4), "little")))
    _w = (lambda a: (lambda t: t.astype(jnp.bfloat16) if jnp.issubdtype(t.dtype, jnp.floating) else t)(jnp.asarray(a)))
    B, Sq, D = 8, 112, 640
    H, Sk, Dh = 32, 512, 192
    return {
        "x": _w((lambda *s: _rng.normal(s) * 0.8)(B, Sq, D)),
        "k_cache": _w((lambda *s: _rng.normal(s) * 0.8)(B, H, Sk, Dh)),
        "v_cache": _w((lambda *s: _rng.normal(s) * 0.05)(B, H, Sk, Dh)),
        "wq": _w((lambda *s: _rng.normal(s) * 0.8)(D, H * Dh) * (D ** -0.5)),
        "wo": _w((lambda *s: _rng.normal(s) * 0.05)(H * Dh, D) * ((H * Dh) ** -0.5)),
    }

def reference(x, k_cache, v_cache, wq, wo):
    B, Sq, D = x.shape
    H, Dh = 32, 192
    q = (lambda x, *d: x.transpose(*d))((x @ wq).reshape(B, Sq, H, Dh), 0, 2, 1, 3)
    scores = jnp.einsum("bhqd,bhkd->bhqk", q, k_cache) * (Dh ** -0.5)
    p = _softmax(scores, axis=-1)
    o = jnp.einsum("bhqk,bhkd->bhqd", p, v_cache)
    return (lambda x, *d: x.transpose(*d))(o, 0, 2, 1, 3).reshape(B, Sq, H * Dh) @ wo
```

```python
import math

import jax
import jax.numpy as jnp
from jax import lax
import jax.experimental.pallas as pl
import jax.experimental.pallas.tpu as pltpu

_NT = (((1,), (1,)), ((), ()))


def _mod(a, n):
    assert n & (n - 1) == 0
    return a % n if isinstance(a, int) else lax.bitwise_and(a, n - 1)


def _div(a, n):
    assert n & (n - 1) == 0
    return a // n if isinstance(a, int) else lax.shift_right_logical(a, n.bit_length() - 1)


@jax.jit
def pallas_standalone__mha_block_cached__near_ridge_kernel(
    x: jax.Array,
    k_cache: jax.Array,
    v_cache: jax.Array,
    wq: jax.Array,
    wo: jax.Array,
):
    B, Sq, D = x.shape
    _, H, Sk, Dh = k_cache.shape
    HP = 2
    G = 2
    W = HP * Dh
    assert Dh == 192 and H % HP == 0 and B % G == 0 and Sq % 16 == 0
    scale = (Dh ** -0.5) * math.log2(math.e)
    kt = jnp.swapaxes(k_cache, 2, 3)
    vt = jnp.swapaxes(v_cache, 2, 3)
    x2 = x.reshape(B * Sq, D)
    nh = H // HP
    bph = B // G
    nblk = nh * bph
    PD = 2
    NS = 4
    assert bph == 4 and NS >= PD + 2
    f32 = jnp.float32
    bf16 = jnp.bfloat16
    GR = G * Sq

    def kernel(x_hbm, wq_hbm, k_hbm, v_hbm, wo_hbm, o_hbm,
               xbuf, wqbuf, kbuf, vbuf, wobuf, qbuf, acc_ref, obuf,
               xsem, wqsem, wosem, ksem, vsem, osem):

        def x_copy(g):
            return pltpu.make_async_copy(
                x_hbm.at[pl.ds(g * GR, GR)], xbuf.at[pl.ds(g * GR, GR)], xsem.at[g])

        def wq_copy(h):
            s = _mod(h, 2)
            return pltpu.make_async_copy(
                wq_hbm.at[:, pl.ds(pl.multiple_of(h * W, 128), W)], wqbuf.at[s], wqsem.at[s])

        def wo_copy(h):
            s = _mod(h, 2)
            return pltpu.make_async_copy(
                wo_hbm.at[pl.ds(pl.multiple_of(h * W, 128), W)], wobuf.at[s], wosem.at[s])

        def kv_src(ref, k):
            return ref.at[pl.ds(_mod(k, bph) * G, G), pl.ds(_div(k, bph) * HP, HP)]

        def k_copy(k):
            s = _mod(k, NS)
            return pltpu.make_async_copy(kv_src(k_hbm, k), kbuf.at[s], ksem.at[s])

        def v_copy(k):
            s = _mod(k, NS)
            return pltpu.make_async_copy(kv_src(v_hbm, k), vbuf.at[s], vsem.at[s])

        def o_copy(g):
            return pltpu.make_async_copy(
                obuf.at[pl.ds(g * GR, GR)], o_hbm.at[pl.ds(g * GR, GR)], osem.at[g])

        zeros64 = jnp.zeros((64, Sk), bf16)

        def row0(k, i):
            return pl.multiple_of(_mod(k, bph) * GR + i * Sq, 16)

        def qproj(k, i):
            q = jnp.dot(xbuf[pl.ds(row0(k, i), Sq), :], wqbuf[_mod(_div(k, bph), 2)],
                        preferred_element_type=f32)
            return (q * scale).astype(bf16)

        def softmax_parts(s):
            m = jnp.max(s, axis=-1, keepdims=True)
            e = jnp.exp2(s - m)
            l = jnp.sum(e, axis=-1, keepdims=True)
            return e.astype(bf16), 1.0 / l

        def qk(k, i):
            s = _mod(k, NS)
            k0 = kbuf[s, i, 0]
            k1 = kbuf[s, i, 1]
            t0, t1, t2 = qbuf[i, :, 0:128], qbuf[i, :, 128:256], qbuf[i, :, 256:384]
            s0 = (jnp.dot(t0, k0[0:128], preferred_element_type=f32)
                  + jnp.dot(t1, jnp.concatenate([k0[128:192], zeros64], axis=0),
                            preferred_element_type=f32))
            s1 = (jnp.dot(t1, jnp.concatenate([zeros64, k1[0:64]], axis=0),
                          preferred_element_type=f32)
                  + jnp.dot(t2, k1[64:192], preferred_element_type=f32))
            return softmax_parts(s0), softmax_parts(s1)

        def pv(k, i, p):
            s = _mod(k, NS)
            (p0, r0), (p1, r1) = p
            ot0 = lax.dot_general(vbuf[s, i, 0], p0, _NT, preferred_element_type=f32)
            ot1 = lax.dot_general(vbuf[s, i, 1], p1, _NT, preferred_element_type=f32)
            ot = jnp.concatenate([ot0 * r0.T, ot1 * r1.T], axis=0)
            return ot.T.astype(bf16)

        def outp(k, i, o):
            acc_ref[pl.ds(row0(k, i), Sq), :] += jnp.dot(
                o, wobuf[_mod(_div(k, bph), 2)], preferred_element_type=f32)

        def emit_out(g):
            r = pl.multiple_of(g * GR, 16)
            obuf[pl.ds(r, GR), :] = acc_ref[pl.ds(r, GR), :].astype(bf16)
            o_copy(g).start()

        def prefetch(k):
            h = _div(k, bph)
            ph = _mod(k, bph)

            @pl.when((ph == 0) & (h + 1 < nh))
            def _():
                wq_copy(h + 1).start()

            @pl.when((ph == 1) & (h + 1 < nh))
            def _():
                wo_copy(h + 1).start()

            @pl.when(k + PD < nblk)
            def _():
                k_copy(k + PD).start()
                v_copy(k + PD).start()

        def block(k, last):
            p0 = qk(k, 0)
            if not last:
                q0 = qproj(k + 1, 0)
            p1 = qk(k, 1)
            if not last:
                prefetch(k)
                q1 = qproj(k + 1, 1)
            o0 = pv(k, 0, p0)
            o1 = pv(k, 1, p1)
            outp(k, 0, o0)
            outp(k, 1, o1)
            if not last:
                qbuf[0] = q0
                qbuf[1] = q1

        x_copy(0).start()
        wq_copy(0).start()
        acc_ref[...] = jnp.zeros(acc_ref.shape, f32)
        x_copy(0).wait()
        k_copy(0).start()
        wq_copy(0).wait()
        v_copy(0).start()
        wo_copy(0).start()
        x_copy(1).start()
        qbuf[0] = qproj(0, 0)
        qbuf[1] = qproj(0, 1)
        k_copy(0).wait()
        k_copy(1).start()
        v_copy(1).start()
        x_copy(2).start()
        x_copy(3).start()

        def body(k, carry):
            h = _div(k, bph)
            ph = _mod(k, bph)

            @pl.when(k > 0)
            def _():
                k_copy(k).wait()

            v_copy(k).wait()

            @pl.when(k + 1 < bph)
            def _():
                x_copy(k + 1).wait()

            @pl.when(ph == 0)
            def _():
                wo_copy(h).wait()

            @pl.when((ph == bph - 1) & (h + 1 < nh))
            def _():
                wq_copy(h + 1).wait()

            @pl.when(k >= nblk - bph + 1)
            def _():
                emit_out(k - (nblk - bph + 1))

            block(k, False)
            return carry

        lax.fori_loop(0, nblk - 1, body, 0)

        kl = nblk - 1
        k_copy(kl).wait()
        v_copy(kl).wait()
        emit_out(bph - 2)
        block(kl, True)
        emit_out(bph - 1)
        for g in range(bph):
            o_copy(g).wait()

    out = pl.pallas_call(
        kernel,
        in_specs=[pl.BlockSpec(memory_space=pl.ANY)] * 5,
        out_specs=pl.BlockSpec(memory_space=pl.ANY),
        out_shape=jax.ShapeDtypeStruct((B * Sq, D), x.dtype),
        scratch_shapes=[
            pltpu.VMEM((B * Sq, D), bf16),
            pltpu.VMEM((2, D, W), bf16),
            pltpu.VMEM((NS, G, HP, Dh, Sk), bf16),
            pltpu.VMEM((NS, G, HP, Dh, Sk), bf16),
            pltpu.VMEM((2, W, D), bf16),
            pltpu.VMEM((G, Sq, W), bf16),
            pltpu.VMEM((B * Sq, D), f32),
            pltpu.VMEM((B * Sq, D), bf16),
            pltpu.SemaphoreType.DMA((bph,)),
            pltpu.SemaphoreType.DMA((2,)),
            pltpu.SemaphoreType.DMA((2,)),
            pltpu.SemaphoreType.DMA((NS,)),
            pltpu.SemaphoreType.DMA((NS,)),
            pltpu.SemaphoreType.DMA((bph,)),
        ],
        compiler_params=pltpu.CompilerParams(
            vmem_limit_bytes=64 * 1024 * 1024,
            disable_bounds_checks=True),
    )(x2, wq, kt, vt, wo)
    return out.reshape(B, Sq, D)
```

```python
import math

import jax
import jax.numpy as jnp
from jax import lax
import jax.experimental.pallas as pl
import jax.experimental.pallas.tpu as pltpu

_NT = (((1,), (1,)), ((), ()))


def _mod(a, n):
    assert n & (n - 1) == 0
    return a % n if isinstance(a, int) else lax.bitwise_and(a, n - 1)


def _div(a, n):
    assert n & (n - 1) == 0
    return a // n if isinstance(a, int) else lax.shift_right_logical(a, n.bit_length() - 1)


@jax.jit
def pallas_standalone__mha_block_cached__near_ridge_kernel(
    x: jax.Array,
    k_cache: jax.Array,
    v_cache: jax.Array,
    wq: jax.Array,
    wo: jax.Array,
):
    B, Sq, D = x.shape
    _, H, Sk, Dh = k_cache.shape
    HP = 2
    G = 2
    W = HP * Dh
    assert Dh == 192 and H % HP == 0 and B % G == 0 and Sq % 16 == 0
    scale = (Dh ** -0.5) * math.log2(math.e)
    kt = jnp.swapaxes(k_cache, 2, 3)
    vt = jnp.swapaxes(v_cache, 2, 3)
    x2 = x.reshape(B * Sq, D)
    nh = H // HP
    bph = B // G
    nblk = nh * bph
    PD = 2
    NS = 4
    assert bph == 4 and NS >= PD + 2 and nh >= 2
    f32 = jnp.float32
    bf16 = jnp.bfloat16
    GR = G * Sq
    nmain = nblk - bph
    kl = nblk - 1

    def kernel(x_hbm, wq_hbm, k_hbm, v_hbm, wo_hbm, o_hbm,
               xbuf, wqbuf, kbuf, vbuf, wobuf, qbuf, acc_ref, obuf,
               xsem, wqsem, wosem, ksem, vsem, osem, lsem):

        def x_copy(g):
            return pltpu.make_async_copy(
                x_hbm.at[pl.ds(g * GR, GR)], xbuf.at[pl.ds(g * GR, GR)], xsem.at[g])

        def wq_copy(h):
            s = _mod(h, 2)
            return pltpu.make_async_copy(
                wq_hbm.at[:, pl.ds(pl.multiple_of(h * W, 128), W)], wqbuf.at[s], wqsem.at[s])

        def wo_copy(h):
            s = _mod(h, 2)
            return pltpu.make_async_copy(
                wo_hbm.at[pl.ds(pl.multiple_of(h * W, 128), W)], wobuf.at[s], wosem.at[s])

        def kv_src(ref, k):
            return ref.at[pl.ds(_mod(k, bph) * G, G), pl.ds(_div(k, bph) * HP, HP)]

        def k_copy(k):
            s = _mod(k, NS)
            return pltpu.make_async_copy(kv_src(k_hbm, k), kbuf.at[s], ksem.at[s])

        def v_copy(k):
            s = _mod(k, NS)
            return pltpu.make_async_copy(kv_src(v_hbm, k), vbuf.at[s], vsem.at[s])

        def vlast_copy(i):
            return pltpu.make_async_copy(
                v_hbm.at[(kl % bph) * G + i, pl.ds((kl // bph) * HP, HP)],
                vbuf.at[kl % NS, i], lsem.at[i])

        def o_copy(r, n, sem):
            return pltpu.make_async_copy(obuf.at[pl.ds(r, n)], o_hbm.at[pl.ds(r, n)], sem)

        zeros64 = jnp.zeros((64, Sk), bf16)

        def row0(g, i):
            return pl.multiple_of(g * GR + i * Sq, 16)

        def qproj(g, i, h):
            q = jnp.dot(xbuf[pl.ds(row0(g, i), Sq), :], wqbuf[_mod(h, 2)],
                        preferred_element_type=f32)
            return (q * scale).astype(bf16)

        def softmax_parts(s):
            m = jnp.max(s, axis=-1, keepdims=True)
            e = jnp.exp2(s - m)
            l = jnp.sum(e, axis=-1, keepdims=True)
            return e.astype(bf16), 1.0 / l

        def qk(k, i):
            s = _mod(k, NS)
            g = _mod(k, bph)
            k0 = kbuf[s, i, 0]
            k1 = kbuf[s, i, 1]
            t0, t1, t2 = qbuf[g, i, :, 0:128], qbuf[g, i, :, 128:256], qbuf[g, i, :, 256:384]
            s0 = (jnp.dot(t0, k0[0:128], preferred_element_type=f32)
                  + jnp.dot(t1, jnp.concatenate([k0[128:192], zeros64], axis=0),
                            preferred_element_type=f32))
            s1 = (jnp.dot(t1, jnp.concatenate([zeros64, k1[0:64]], axis=0),
                          preferred_element_type=f32)
                  + jnp.dot(t2, k1[64:192], preferred_element_type=f32))
            return softmax_parts(s0), softmax_parts(s1)

        def pv(k, i, p):
            s = _mod(k, NS)
            (p0, r0), (p1, r1) = p
            ot0 = lax.dot_general(vbuf[s, i, 0], p0, _NT, preferred_element_type=f32)
            ot1 = lax.dot_general(vbuf[s, i, 1], p1, _NT, preferred_element_type=f32)
            ot = jnp.concatenate([ot0 * r0.T, ot1 * r1.T], axis=0)
            return ot.T.astype(bf16)

        def outp(k, i, o):
            acc_ref[pl.ds(row0(_mod(k, bph), i), Sq), :] += jnp.dot(
                o, wobuf[_mod(_div(k, bph), 2)], preferred_element_type=f32)

        def emit_rows(r, n, sem):
            obuf[pl.ds(r, n), :] = acc_ref[pl.ds(r, n), :].astype(bf16)
            o_copy(r, n, sem).start()

        x_copy(0).start()
        wq_copy(0).start()
        acc_ref[...] = jnp.zeros(acc_ref.shape, f32)
        x_copy(0).wait()
        x_copy(1).start()
        x_copy(2).start()
        x_copy(3).start()
        wq_copy(0).wait()
        k_copy(0).start()
        v_copy(0).start()
        qbuf[0, 0] = qproj(0, 0, 0)
        qbuf[0, 1] = qproj(0, 1, 0)
        x_copy(1).wait()
        wo_copy(0).start()
        wq_copy(1).start()
        qbuf[1, 0] = qproj(1, 0, 0)
        qbuf[1, 1] = qproj(1, 1, 0)
        x_copy(2).wait()
        k_copy(1).start()
        v_copy(1).start()
        qbuf[2, 0] = qproj(2, 0, 0)
        qbuf[2, 1] = qproj(2, 1, 0)
        x_copy(3).wait()
        qbuf[3, 0] = qproj(3, 0, 0)
        qbuf[3, 1] = qproj(3, 1, 0)

        def body(k, carry):
            h = _div(k, bph)
            ph = _mod(k, bph)
            k_copy(k).wait()
            v_copy(k).wait()

            @pl.when(ph == 0)
            def _():
                wo_copy(h).wait()
                wq_copy(h + 1).wait()

            p0 = qk(k, 0)
            q0 = qproj(ph, 0, h + 1)
            p1 = qk(k, 1)

            @pl.when((ph == 0) & (h + 2 < nh))
            def _():
                wq_copy(h + 2).start()

            @pl.when(ph == 1)
            def _():
                wo_copy(h + 1).start()

            k_copy(k + PD).start()
            v_copy(k + PD).start()

            q1 = qproj(ph, 1, h + 1)
            o0 = pv(k, 0, p0)
            o1 = pv(k, 1, p1)
            outp(k, 0, o0)
            outp(k, 1, o1)
            qbuf[ph, 0] = q0
            qbuf[ph, 1] = q1
            return carry

        lax.fori_loop(0, nmain, body, 0)

        def tail(k, carry):
            ph = _mod(k, bph)
            k_copy(k).wait()
            v_copy(k).wait()

            @pl.when(ph == 0)
            def _():
                wo_copy(nh - 1).wait()

            @pl.when(k + PD < kl)
            def _():
                k_copy(k + PD).start()
                v_copy(k + PD).start()

            @pl.when(k + PD == kl)
            def _():
                k_copy(kl).start()
                vlast_copy(0).start()
                vlast_copy(1).start()

            p0 = qk(k, 0)
            p1 = qk(k, 1)
            o0 = pv(k, 0, p0)
            o1 = pv(k, 1, p1)
            outp(k, 0, o0)
            outp(k, 1, o1)
            emit_rows(pl.multiple_of(ph * GR, 16), GR, osem.at[ph])
            return carry

        lax.fori_loop(nmain, kl, tail, 0)

        rl = (bph - 1) * GR
        k_copy(kl).wait()
        p0 = qk(kl, 0)
        p1 = qk(kl, 1)
        vlast_copy(0).wait()
        outp(kl, 0, pv(kl, 0, p0))
        emit_rows(rl, Sq, osem.at[bph - 1])
        vlast_copy(1).wait()
        outp(kl, 1, pv(kl, 1, p1))
        emit_rows(rl + Sq, Sq, osem.at[bph])
        for g in range(bph - 1):
            o_copy(g * GR, GR, osem.at[g]).wait()
        o_copy(rl, Sq, osem.at[bph - 1]).wait()
        o_copy(rl + Sq, Sq, osem.at[bph]).wait()

    out = pl.pallas_call(
        kernel,
        in_specs=[pl.BlockSpec(memory_space=pl.ANY)] * 5,
        out_specs=pl.BlockSpec(memory_space=pl.ANY),
        out_shape=jax.ShapeDtypeStruct((B * Sq, D), x.dtype),
        scratch_shapes=[
            pltpu.VMEM((B * Sq, D), bf16),
            pltpu.VMEM((2, D, W), bf16),
            pltpu.VMEM((NS, G, HP, Dh, Sk), bf16),
            pltpu.VMEM((NS, G, HP, Dh, Sk), bf16),
            pltpu.VMEM((2, W, D), bf16),
            pltpu.VMEM((bph, G, Sq, W), bf16),
            pltpu.VMEM((B * Sq, D), f32),
            pltpu.VMEM((B * Sq, D), bf16),
            pltpu.SemaphoreType.DMA((bph,)),
            pltpu.SemaphoreType.DMA((2,)),
            pltpu.SemaphoreType.DMA((2,)),
            pltpu.SemaphoreType.DMA((NS,)),
            pltpu.SemaphoreType.DMA((NS,)),
            pltpu.SemaphoreType.DMA((bph + 1,)),
            pltpu.SemaphoreType.DMA((G,)),
        ],
        compiler_params=pltpu.CompilerParams(
            vmem_limit_bytes=64 * 1024 * 1024,
            disable_bounds_checks=True),
    )(x2, wq, kt, vt, wo)
    return out.reshape(B, Sq, D)
```

```python
import math

import jax
import jax.numpy as jnp
from jax import lax
import jax.experimental.pallas as pl
import jax.experimental.pallas.tpu as pltpu

_NT = (((1,), (1,)), ((), ()))


def _mod(a, n):
    assert n & (n - 1) == 0
    return a % n if isinstance(a, int) else lax.bitwise_and(a, n - 1)


def _div(a, n):
    assert n & (n - 1) == 0
    return a // n if isinstance(a, int) else lax.shift_right_logical(a, n.bit_length() - 1)


@jax.jit
def pallas_standalone__mha_block_cached__near_ridge_kernel(
    x: jax.Array,
    k_cache: jax.Array,
    v_cache: jax.Array,
    wq: jax.Array,
    wo: jax.Array,
):
    B, Sq, D = x.shape
    _, H, Sk, Dh = k_cache.shape
    HP = 2
    G = 2
    W = HP * Dh
    assert Dh == 192 and H % HP == 0 and B % G == 0 and Sq % 16 == 0
    scale = (Dh ** -0.5) * math.log2(math.e)
    kt = jnp.swapaxes(k_cache, 2, 3)
    vt = jnp.swapaxes(v_cache, 2, 3)
    x2 = x.reshape(B * Sq, D)
    nh = H // HP
    bph = B // G
    nblk = nh * bph
    PD = 2
    NS = 4
    assert bph == 4 and NS >= PD + 2 and nh >= 2
    f32 = jnp.float32
    bf16 = jnp.bfloat16
    GR = G * Sq
    nmain = nblk - bph
    kl = nblk - 1

    def kernel(x_hbm, wq_hbm, k_hbm, v_hbm, wo_hbm, o_hbm,
               xbuf, wqbuf, kbuf, vbuf, wobuf, qbuf, acc_ref, obuf,
               xsem, wqsem, wosem, ksem, vsem, osem, lsem):

        def x_copy(g):
            return pltpu.make_async_copy(
                x_hbm.at[pl.ds(g * GR, GR)], xbuf.at[pl.ds(g * GR, GR)], xsem.at[g])

        def wq_copy(h):
            s = _mod(h, 2)
            return pltpu.make_async_copy(
                wq_hbm.at[:, pl.ds(pl.multiple_of(h * W, 128), W)], wqbuf.at[s], wqsem.at[s])

        def wo_copy(h):
            s = _mod(h, 2)
            return pltpu.make_async_copy(
                wo_hbm.at[pl.ds(pl.multiple_of(h * W, 128), W)], wobuf.at[s], wosem.at[s])

        def kv_src(ref, k):
            return ref.at[pl.ds(_mod(k, bph) * G, G), pl.ds(_div(k, bph) * HP, HP)]

        def k_copy(k):
            s = _mod(k, NS)
            return pltpu.make_async_copy(kv_src(k_hbm, k), kbuf.at[s], ksem.at[s])

        def v_copy(k):
            s = _mod(k, NS)
            return pltpu.make_async_copy(kv_src(v_hbm, k), vbuf.at[s], vsem.at[s])

        def vlast_copy(i):
            return pltpu.make_async_copy(
                v_hbm.at[(kl % bph) * G + i, pl.ds((kl // bph) * HP, HP)],
                vbuf.at[kl % NS, i], lsem.at[i])

        def o_copy(r, n, sem):
            return pltpu.make_async_copy(obuf.at[pl.ds(r, n)], o_hbm.at[pl.ds(r, n)], sem)

        zeros64 = jnp.zeros((64, Sk), bf16)

        def row0(g, i):
            return pl.multiple_of(g * GR + i * Sq, 16)

        def qproj(g, i, h):
            q = jnp.dot(xbuf[pl.ds(row0(g, i), Sq), :], wqbuf[_mod(h, 2)],
                        preferred_element_type=f32)
            return (q * scale).astype(bf16)

        def softmax_parts(s):
            m = jnp.max(s, axis=-1, keepdims=True)
            e = jnp.exp2(s - m)
            l = jnp.sum(e, axis=-1, keepdims=True)
            return e.astype(bf16), 1.0 / l

        def qk(k, i):
            s = _mod(k, NS)
            g = _mod(k, bph)
            k0 = kbuf[s, i, 0]
            k1 = kbuf[s, i, 1]
            t0, t1, t2 = qbuf[g, i, :, 0:128], qbuf[g, i, :, 128:256], qbuf[g, i, :, 256:384]
            s0 = (jnp.dot(t0, k0[0:128], preferred_element_type=f32)
                  + jnp.dot(t1, jnp.concatenate([k0[128:192], zeros64], axis=0),
                            preferred_element_type=f32))
            s1 = (jnp.dot(t1, jnp.concatenate([zeros64, k1[0:64]], axis=0),
                          preferred_element_type=f32)
                  + jnp.dot(t2, k1[64:192], preferred_element_type=f32))
            return softmax_parts(s0), softmax_parts(s1)

        def pv(k, i, p):
            s = _mod(k, NS)
            (p0, r0), (p1, r1) = p
            ot0 = lax.dot_general(vbuf[s, i, 0], p0, _NT, preferred_element_type=f32)
            ot1 = lax.dot_general(vbuf[s, i, 1], p1, _NT, preferred_element_type=f32)
            ot = jnp.concatenate([ot0 * r0.T, ot1 * r1.T], axis=0)
            return ot.T.astype(bf16)

        def outp(k, i, o):
            acc_ref[pl.ds(row0(_mod(k, bph), i), Sq), :] += jnp.dot(
                o, wobuf[_mod(_div(k, bph), 2)], preferred_element_type=f32)

        def emit_rows(r, n, sem):
            obuf[pl.ds(r, n), :] = acc_ref[pl.ds(r, n), :].astype(bf16)
            o_copy(r, n, sem).start()

        x_copy(0).start()
        wq_copy(0).start()
        acc_ref[...] = jnp.zeros(acc_ref.shape, f32)
        x_copy(0).wait()
        x_copy(1).start()
        x_copy(2).start()
        x_copy(3).start()
        wq_copy(0).wait()
        k_copy(0).start()
        v_copy(0).start()
        qbuf[0, 0] = qproj(0, 0, 0)
        qbuf[0, 1] = qproj(0, 1, 0)
        x_copy(1).wait()
        wo_copy(0).start()
        wq_copy(1).start()
        qbuf[1, 0] = qproj(1, 0, 0)
        qbuf[1, 1] = qproj(1, 1, 0)
        x_copy(2).wait()
        k_copy(1).start()
        v_copy(1).start()
        qbuf[2, 0] = qproj(2, 0, 0)
        qbuf[2, 1] = qproj(2, 1, 0)
        x_copy(3).wait()
        qbuf[3, 0] = qproj(3, 0, 0)
        qbuf[3, 1] = qproj(3, 1, 0)

        def body(k, carry):
            h = _div(k, bph)
            ph = _mod(k, bph)
            k_copy(k).wait()
            v_copy(k).wait()

            @pl.when(ph == 0)
            def _():
                wo_copy(h).wait()
                wq_copy(h + 1).wait()

            p0 = qk(k, 0)
            q0 = qproj(ph, 0, h + 1)
            p1 = qk(k, 1)

            @pl.when((ph == 0) & (h + 2 < nh))
            def _():
                wq_copy(h + 2).start()

            @pl.when(ph == 1)
            def _():
                wo_copy(h + 1).start()

            k_copy(k + PD).start()
            v_copy(k + PD).start()

            q1 = qproj(ph, 1, h + 1)
            o0 = pv(k, 0, p0)
            o1 = pv(k, 1, p1)
            outp(k, 0, o0)
            outp(k, 1, o1)
            qbuf[ph, 0] = q0
            qbuf[ph, 1] = q1
            return carry

        lax.fori_loop(0, nmain, body, 0)

        def tail(k, carry):
            ph = _mod(k, bph)
            k_copy(k).wait()
            v_copy(k).wait()

            @pl.when(ph == 0)
            def _():
                wo_copy(nh - 1).wait()

            @pl.when(k + PD < kl)
            def _():
                k_copy(k + PD).start()
                v_copy(k + PD).start()

            @pl.when(k + PD == kl)
            def _():
                k_copy(kl).start()
                vlast_copy(0).start()
                vlast_copy(1).start()

            p0 = qk(k, 0)
            p1 = qk(k, 1)
            o0 = pv(k, 0, p0)
            o1 = pv(k, 1, p1)
            outp(k, 0, o0)
            outp(k, 1, o1)
            r = pl.multiple_of(ph * GR, 16)
            obuf[pl.ds(r, GR), :] = acc_ref[pl.ds(r, GR), :].astype(bf16)
            return carry

        lax.fori_loop(nmain, kl, tail, 0)

        rl = (bph - 1) * GR
        k_copy(kl).wait()
        o_copy(0, rl, osem.at[0]).start()
        p0 = qk(kl, 0)
        p1 = qk(kl, 1)
        vlast_copy(0).wait()
        outp(kl, 0, pv(kl, 0, p0))
        emit_rows(rl, Sq, osem.at[1])
        vlast_copy(1).wait()
        outp(kl, 1, pv(kl, 1, p1))
        emit_rows(rl + Sq, Sq, osem.at[2])
        o_copy(0, rl, osem.at[0]).wait()
        o_copy(rl, Sq, osem.at[1]).wait()
        o_copy(rl + Sq, Sq, osem.at[2]).wait()

    out = pl.pallas_call(
        kernel,
        in_specs=[pl.BlockSpec(memory_space=pl.ANY)] * 5,
        out_specs=pl.BlockSpec(memory_space=pl.ANY),
        out_shape=jax.ShapeDtypeStruct((B * Sq, D), x.dtype),
        scratch_shapes=[
            pltpu.VMEM((B * Sq, D), bf16),
            pltpu.VMEM((2, D, W), bf16),
            pltpu.VMEM((NS, G, HP, Dh, Sk), bf16),
            pltpu.VMEM((NS, G, HP, Dh, Sk), bf16),
            pltpu.VMEM((2, W, D), bf16),
            pltpu.VMEM((bph, G, Sq, W), bf16),
            pltpu.VMEM((B * Sq, D), f32),
            pltpu.VMEM((B * Sq, D), bf16),
            pltpu.SemaphoreType.DMA((bph,)),
            pltpu.SemaphoreType.DMA((2,)),
            pltpu.SemaphoreType.DMA((2,)),
            pltpu.SemaphoreType.DMA((NS,)),
            pltpu.SemaphoreType.DMA((NS,)),
            pltpu.SemaphoreType.DMA((3,)),
            pltpu.SemaphoreType.DMA((G,)),
        ],
        compiler_params=pltpu.CompilerParams(vmem_limit_bytes=64 * 1024 * 1024),
    )(x2, wq, kt, vt, wo)
    return out.reshape(B, Sq, D)
```

```python
import math

import jax
import jax.numpy as jnp
from jax import lax
import jax.experimental.pallas as pl
import jax.experimental.pallas.tpu as pltpu

_NT = (((1,), (1,)), ((), ()))


def _mod(a, n):
    assert n & (n - 1) == 0
    return a % n if isinstance(a, int) else lax.bitwise_and(a, n - 1)


def _div(a, n):
    assert n & (n - 1) == 0
    return a // n if isinstance(a, int) else lax.shift_right_logical(a, n.bit_length() - 1)


@jax.jit
def pallas_standalone__mha_block_cached__near_ridge_kernel(
    x: jax.Array,
    k_cache: jax.Array,
    v_cache: jax.Array,
    wq: jax.Array,
    wo: jax.Array,
):
    B, Sq, D = x.shape
    _, H, Sk, Dh = k_cache.shape
    HP = 2
    G = 2
    W = HP * Dh
    assert Dh == 192 and H % HP == 0 and B % G == 0 and Sq % 16 == 0
    scale = (Dh ** -0.5) * math.log2(math.e)
    kt = jnp.swapaxes(k_cache, 2, 3)
    vt = jnp.swapaxes(v_cache, 2, 3)
    x2 = x.reshape(B * Sq, D)
    nh = H // HP
    bph = B // G
    nblk = nh * bph
    PD = 2
    NS = 4
    assert bph == 4 and NS >= PD + 2 and nh >= 2
    f32 = jnp.float32
    bf16 = jnp.bfloat16
    GR = G * Sq
    nmain = nblk - bph
    kl = nblk - 1

    def kernel(x_hbm, wq_hbm, k_hbm, v_hbm, wo_hbm, o_hbm,
               xbuf, wqbuf, kbuf, vbuf, wobuf, qbuf, acc_ref, obuf,
               xsem, wqsem, wosem, ksem, vsem, osem):

        def x_copy(g):
            return pltpu.make_async_copy(
                x_hbm.at[pl.ds(g * GR, GR)], xbuf.at[pl.ds(g * GR, GR)], xsem.at[g])

        def wq_copy(h):
            s = _mod(h, 2)
            return pltpu.make_async_copy(
                wq_hbm.at[:, pl.ds(pl.multiple_of(h * W, 128), W)], wqbuf.at[s], wqsem.at[s])

        def wo_copy(h):
            s = _mod(h, 2)
            return pltpu.make_async_copy(
                wo_hbm.at[pl.ds(pl.multiple_of(h * W, 128), W)], wobuf.at[s], wosem.at[s])

        def kv_src(ref, k):
            return ref.at[pl.ds(_mod(k, bph) * G, G), pl.ds(_div(k, bph) * HP, HP)]

        def k_copy(k):
            s = _mod(k, NS)
            return pltpu.make_async_copy(kv_src(k_hbm, k), kbuf.at[s], ksem.at[s])

        def v_copy(k):
            s = _mod(k, NS)
            return pltpu.make_async_copy(kv_src(v_hbm, k), vbuf.at[s], vsem.at[s])

        def o_copy(r, n, sem):
            return pltpu.make_async_copy(obuf.at[pl.ds(r, n)], o_hbm.at[pl.ds(r, n)], sem)

        zeros64 = jnp.zeros((64, Sk), bf16)

        def row0(g, i):
            return pl.multiple_of(g * GR + i * Sq, 16)

        def qproj(g, i, h):
            q = jnp.dot(xbuf[pl.ds(row0(g, i), Sq), :], wqbuf[_mod(h, 2)],
                        preferred_element_type=f32)
            return (q * scale).astype(bf16)

        def softmax_parts(s):
            m = jnp.max(s, axis=-1, keepdims=True)
            e = jnp.exp2(s - m)
            l = jnp.sum(e, axis=-1, keepdims=True)
            return e.astype(bf16), 1.0 / l

        def qk(k, i):
            s = _mod(k, NS)
            g = _mod(k, bph)
            k0 = kbuf[s, i, 0]
            k1 = kbuf[s, i, 1]
            t0, t1, t2 = qbuf[g, i, :, 0:128], qbuf[g, i, :, 128:256], qbuf[g, i, :, 256:384]
            s0 = (jnp.dot(t0, k0[0:128], preferred_element_type=f32)
                  + jnp.dot(t1, jnp.concatenate([k0[128:192], zeros64], axis=0),
                            preferred_element_type=f32))
            s1 = (jnp.dot(t1, jnp.concatenate([zeros64, k1[0:64]], axis=0),
                          preferred_element_type=f32)
                  + jnp.dot(t2, k1[64:192], preferred_element_type=f32))
            return softmax_parts(s0), softmax_parts(s1)

        def pv(k, i, p):
            s = _mod(k, NS)
            (p0, r0), (p1, r1) = p
            ot0 = lax.dot_general(vbuf[s, i, 0], p0, _NT, preferred_element_type=f32)
            ot1 = lax.dot_general(vbuf[s, i, 1], p1, _NT, preferred_element_type=f32)
            ot = jnp.concatenate([ot0 * r0.T, ot1 * r1.T], axis=0)
            return ot.T.astype(bf16)

        def outp(k, i, o):
            acc_ref[pl.ds(row0(_mod(k, bph), i), Sq), :] += jnp.dot(
                o, wobuf[_mod(_div(k, bph), 2)], preferred_element_type=f32)

        def emit_rows(r, n, sem):
            obuf[pl.ds(r, n), :] = acc_ref[pl.ds(r, n), :].astype(bf16)
            o_copy(r, n, sem).start()

        x_copy(0).start()
        wq_copy(0).start()
        acc_ref[...] = jnp.zeros(acc_ref.shape, f32)
        x_copy(0).wait()
        x_copy(1).start()
        x_copy(2).start()
        x_copy(3).start()
        wq_copy(0).wait()
        k_copy(0).start()
        v_copy(0).start()
        qbuf[0, 0] = qproj(0, 0, 0)
        qbuf[0, 1] = qproj(0, 1, 0)
        x_copy(1).wait()
        wo_copy(0).start()
        wq_copy(1).start()
        qbuf[1, 0] = qproj(1, 0, 0)
        qbuf[1, 1] = qproj(1, 1, 0)
        x_copy(2).wait()
        k_copy(1).start()
        v_copy(1).start()
        qbuf[2, 0] = qproj(2, 0, 0)
        qbuf[2, 1] = qproj(2, 1, 0)
        x_copy(3).wait()
        qbuf[3, 0] = qproj(3, 0, 0)
        qbuf[3, 1] = qproj(3, 1, 0)

        def body(k, carry):
            h = _div(k, bph)
            ph = _mod(k, bph)
            k_copy(k).wait()
            v_copy(k).wait()

            @pl.when(ph == 0)
            def _():
                wo_copy(h).wait()
                wq_copy(h + 1).wait()

            p0 = qk(k, 0)
            q0 = qproj(ph, 0, h + 1)
            p1 = qk(k, 1)

            @pl.when((ph == 0) & (h + 2 < nh))
            def _():
                wq_copy(h + 2).start()

            @pl.when(ph == 1)
            def _():
                wo_copy(h + 1).start()

            k_copy(k + PD).start()
            v_copy(k + PD).start()

            q1 = qproj(ph, 1, h + 1)
            o0 = pv(k, 0, p0)
            o1 = pv(k, 1, p1)
            outp(k, 0, o0)
            outp(k, 1, o1)
            qbuf[ph, 0] = q0
            qbuf[ph, 1] = q1
            return carry

        lax.fori_loop(0, nmain, body, 0)

        def tail(k, carry):
            ph = _mod(k, bph)
            k_copy(k).wait()
            v_copy(k).wait()

            @pl.when(ph == 0)
            def _():
                wo_copy(nh - 1).wait()

            @pl.when(k + PD < nblk)
            def _():
                k_copy(k + PD).start()
                v_copy(k + PD).start()

            p0 = qk(k, 0)
            p1 = qk(k, 1)
            o0 = pv(k, 0, p0)
            o1 = pv(k, 1, p1)
            outp(k, 0, o0)
            outp(k, 1, o1)
            r = pl.multiple_of(ph * GR, 16)
            obuf[pl.ds(r, GR), :] = acc_ref[pl.ds(r, GR), :].astype(bf16)
            return carry

        lax.fori_loop(nmain, kl, tail, 0)

        rl = (bph - 1) * GR
        k_copy(kl).wait()
        v_copy(kl).wait()
        o_copy(0, rl, osem.at[0]).start()
        p0 = qk(kl, 0)
        p1 = qk(kl, 1)
        o0 = pv(kl, 0, p0)
        o1 = pv(kl, 1, p1)
        outp(kl, 0, o0)
        emit_rows(rl, Sq, osem.at[1])
        outp(kl, 1, o1)
        emit_rows(rl + Sq, Sq, osem.at[2])
        o_copy(0, rl, osem.at[0]).wait()
        o_copy(rl, Sq, osem.at[1]).wait()
        o_copy(rl + Sq, Sq, osem.at[2]).wait()

    out = pl.pallas_call(
        kernel,
        in_specs=[pl.BlockSpec(memory_space=pl.ANY)] * 5,
        out_specs=pl.BlockSpec(memory_space=pl.ANY),
        out_shape=jax.ShapeDtypeStruct((B * Sq, D), x.dtype),
        scratch_shapes=[
            pltpu.VMEM((B * Sq, D), bf16),
            pltpu.VMEM((2, D, W), bf16),
            pltpu.VMEM((NS, G, HP, Dh, Sk), bf16),
            pltpu.VMEM((NS, G, HP, Dh, Sk), bf16),
            pltpu.VMEM((2, W, D), bf16),
            pltpu.VMEM((bph, G, Sq, W), bf16),
            pltpu.VMEM((B * Sq, D), f32),
            pltpu.VMEM((B * Sq, D), bf16),
            pltpu.SemaphoreType.DMA((bph,)),
            pltpu.SemaphoreType.DMA((2,)),
            pltpu.SemaphoreType.DMA((2,)),
            pltpu.SemaphoreType.DMA((NS,)),
            pltpu.SemaphoreType.DMA((NS,)),
            pltpu.SemaphoreType.DMA((3,)),
        ],
        compiler_params=pltpu.CompilerParams(vmem_limit_bytes=64 * 1024 * 1024),
    )(x2, wq, kt, vt, wo)
    return out.reshape(B, Sq, D)
```

```python
import math

import jax
import jax.numpy as jnp
from jax import lax
import jax.experimental.pallas as pl
import jax.experimental.pallas.tpu as pltpu

_NT = (((1,), (1,)), ((), ()))


def _mod(a, n):
    assert n & (n - 1) == 0
    return a % n if isinstance(a, int) else lax.bitwise_and(a, n - 1)


def _div(a, n):
    assert n & (n - 1) == 0
    return a // n if isinstance(a, int) else lax.shift_right_logical(a, n.bit_length() - 1)


@jax.jit
def pallas_standalone__mha_block_cached__near_ridge_kernel(
    x: jax.Array,
    k_cache: jax.Array,
    v_cache: jax.Array,
    wq: jax.Array,
    wo: jax.Array,
):
    B, Sq, D = x.shape
    _, H, Sk, Dh = k_cache.shape
    HP = 2
    G = 2
    W = HP * Dh
    assert Dh == 192 and H % HP == 0 and B % G == 0 and Sq % 16 == 0
    scale = (Dh ** -0.5) * math.log2(math.e)
    kt = jnp.swapaxes(k_cache, 2, 3)
    vt = jnp.swapaxes(v_cache, 2, 3)
    x2 = x.reshape(B * Sq, D)
    nh = H // HP
    bph = B // G
    nblk = nh * bph
    PD = 2
    NS = 4
    assert bph == 4 and NS >= PD + 2 and nh >= 2
    f32 = jnp.float32
    bf16 = jnp.bfloat16
    GR = G * Sq
    nmain = nblk - bph
    kl = nblk - 1

    def kernel(x_hbm, wq_hbm, k_hbm, v_hbm, wo_hbm, o_hbm,
               xbuf, wqbuf, kbuf, vbuf, wobuf, qbuf, acc_ref, obuf,
               xsem, wqsem, wosem, ksem, vsem, osem):

        x_copy = pltpu.make_async_copy(x_hbm, xbuf, xsem.at[0])

        def wq_copy(h):
            s = _mod(h, 2)
            return pltpu.make_async_copy(
                wq_hbm.at[:, pl.ds(pl.multiple_of(h * W, 128), W)], wqbuf.at[s], wqsem.at[s])

        def wo_copy(h):
            s = _mod(h, 2)
            return pltpu.make_async_copy(
                wo_hbm.at[pl.ds(pl.multiple_of(h * W, 128), W)], wobuf.at[s], wosem.at[s])

        def kv_src(ref, k):
            return ref.at[pl.ds(_mod(k, bph) * G, G), pl.ds(_div(k, bph) * HP, HP)]

        def k_copy(k):
            s = _mod(k, NS)
            return pltpu.make_async_copy(kv_src(k_hbm, k), kbuf.at[s], ksem.at[s])

        def v_copy(k):
            s = _mod(k, NS)
            return pltpu.make_async_copy(kv_src(v_hbm, k), vbuf.at[s], vsem.at[s])

        def o_copy(r, n, sem):
            return pltpu.make_async_copy(obuf.at[pl.ds(r, n)], o_hbm.at[pl.ds(r, n)], sem)

        zeros64 = jnp.zeros((64, Sk), bf16)

        def row0(g, i):
            return pl.multiple_of(g * GR + i * Sq, 16)

        def qproj(g, i, h):
            q = jnp.dot(xbuf[pl.ds(row0(g, i), Sq), :], wqbuf[_mod(h, 2)],
                        preferred_element_type=f32)
            return (q * scale).astype(bf16)

        def softmax_parts(s):
            m = jnp.max(s, axis=-1, keepdims=True)
            e = jnp.exp2(s - m)
            l = jnp.sum(e, axis=-1, keepdims=True)
            return e.astype(bf16), 1.0 / l

        def qk(k, i):
            s = _mod(k, NS)
            g = _mod(k, bph)
            k0 = kbuf[s, i, 0]
            k1 = kbuf[s, i, 1]
            t0, t1, t2 = qbuf[g, i, :, 0:128], qbuf[g, i, :, 128:256], qbuf[g, i, :, 256:384]
            s0 = (jnp.dot(t0, k0[0:128], preferred_element_type=f32)
                  + jnp.dot(t1, jnp.concatenate([k0[128:192], zeros64], axis=0),
                            preferred_element_type=f32))
            s1 = (jnp.dot(t1, jnp.concatenate([zeros64, k1[0:64]], axis=0),
                          preferred_element_type=f32)
                  + jnp.dot(t2, k1[64:192], preferred_element_type=f32))
            return softmax_parts(s0), softmax_parts(s1)

        def pv(k, i, p):
            s = _mod(k, NS)
            (p0, r0), (p1, r1) = p
            ot0 = lax.dot_general(vbuf[s, i, 0], p0, _NT, preferred_element_type=f32)
            ot1 = lax.dot_general(vbuf[s, i, 1], p1, _NT, preferred_element_type=f32)
            ot = jnp.concatenate([ot0 * r0.T, ot1 * r1.T], axis=0)
            return ot.T.astype(bf16)

        def outp(k, i, o):
            acc_ref[pl.ds(row0(_mod(k, bph), i), Sq), :] += jnp.dot(
                o, wobuf[_mod(_div(k, bph), 2)], preferred_element_type=f32)

        def emit_rows(r, n, sem):
            obuf[pl.ds(r, n), :] = acc_ref[pl.ds(r, n), :].astype(bf16)
            o_copy(r, n, sem).start()

        wq_copy(0).start()
        x_copy.start()
        acc_ref[...] = jnp.zeros(acc_ref.shape, f32)
        wq_copy(0).wait()
        k_copy(0).start()
        v_copy(0).start()
        x_copy.wait()
        wo_copy(0).start()
        wq_copy(1).start()
        k_copy(1).start()
        v_copy(1).start()
        for g in range(bph):
            for i in range(G):
                qbuf[g, i] = qproj(g, i, 0)

        def body(k, carry):
            h = _div(k, bph)
            ph = _mod(k, bph)
            k_copy(k).wait()
            v_copy(k).wait()

            @pl.when(ph == 0)
            def _():
                wo_copy(h).wait()
                wq_copy(h + 1).wait()

            p0 = qk(k, 0)
            q0 = qproj(ph, 0, h + 1)
            p1 = qk(k, 1)

            @pl.when((ph == 0) & (h + 2 < nh))
            def _():
                wq_copy(h + 2).start()

            @pl.when(ph == 1)
            def _():
                wo_copy(h + 1).start()

            k_copy(k + PD).start()
            v_copy(k + PD).start()

            q1 = qproj(ph, 1, h + 1)
            o0 = pv(k, 0, p0)
            o1 = pv(k, 1, p1)
            outp(k, 0, o0)
            outp(k, 1, o1)
            qbuf[ph, 0] = q0
            qbuf[ph, 1] = q1
            return carry

        lax.fori_loop(0, nmain, body, 0)

        def tail(k, carry):
            ph = _mod(k, bph)
            k_copy(k).wait()
            v_copy(k).wait()

            @pl.when(ph == 0)
            def _():
                wo_copy(nh - 1).wait()

            @pl.when(k + PD < nblk)
            def _():
                k_copy(k + PD).start()
                v_copy(k + PD).start()

            p0 = qk(k, 0)
            p1 = qk(k, 1)
            o0 = pv(k, 0, p0)
            o1 = pv(k, 1, p1)
            outp(k, 0, o0)
            outp(k, 1, o1)
            r = pl.multiple_of(ph * GR, 16)
            obuf[pl.ds(r, GR), :] = acc_ref[pl.ds(r, GR), :].astype(bf16)
            return carry

        lax.fori_loop(nmain, kl, tail, 0)

        rl = (bph - 1) * GR
        k_copy(kl).wait()
        v_copy(kl).wait()
        o_copy(0, rl, osem.at[0]).start()
        p0 = qk(kl, 0)
        p1 = qk(kl, 1)
        o0 = pv(kl, 0, p0)
        o1 = pv(kl, 1, p1)
        outp(kl, 0, o0)
        emit_rows(rl, Sq, osem.at[1])
        outp(kl, 1, o1)
        emit_rows(rl + Sq, Sq, osem.at[2])
        o_copy(0, rl, osem.at[0]).wait()
        o_copy(rl, Sq, osem.at[1]).wait()
        o_copy(rl + Sq, Sq, osem.at[2]).wait()

    out = pl.pallas_call(
        kernel,
        in_specs=[pl.BlockSpec(memory_space=pl.ANY)] * 5,
        out_specs=pl.BlockSpec(memory_space=pl.ANY),
        out_shape=jax.ShapeDtypeStruct((B * Sq, D), x.dtype),
        scratch_shapes=[
            pltpu.VMEM((B * Sq, D), bf16),
            pltpu.VMEM((2, D, W), bf16),
            pltpu.VMEM((NS, G, HP, Dh, Sk), bf16),
            pltpu.VMEM((NS, G, HP, Dh, Sk), bf16),
            pltpu.VMEM((2, W, D), bf16),
            pltpu.VMEM((bph, G, Sq, W), bf16),
            pltpu.VMEM((B * Sq, D), f32),
            pltpu.VMEM((B * Sq, D), bf16),
            pltpu.SemaphoreType.DMA((1,)),
            pltpu.SemaphoreType.DMA((2,)),
            pltpu.SemaphoreType.DMA((2,)),
            pltpu.SemaphoreType.DMA((NS,)),
            pltpu.SemaphoreType.DMA((NS,)),
            pltpu.SemaphoreType.DMA((3,)),
        ],
        compiler_params=pltpu.CompilerParams(vmem_limit_bytes=64 * 1024 * 1024),
    )(x2, wq, kt, vt, wo)
    return out.reshape(B, Sq, D)
```
